```python
import jax
import jax.numpy as jnp

def _softmax(x, axis=-1):
    return jax.nn.softmax(x, axis=axis)

def _gelu(x):
    return jax.nn.gelu(x, approximate=True)

def _silu(x):
    return jax.nn.silu(x)

def _sigmoid(x):
    return jax.nn.sigmoid(x)

def _layernorm(x, axis=-1, eps=1e-05):
    m = jnp.mean(x, axis=axis, keepdims=True)
    v = jnp.var(x, axis=axis, keepdims=True)
    return (x - m) / jnp.sqrt(v + eps)

def _scatter_add(tgt, idx, src, axis=0):
    return tgt.at[idx].add(src)

def _segment_sum(src, seg, n):
    return jax.ops.segment_sum(src, seg, n)

class _Rng:

    def __init__(self, key):
        self._k = key

    def _next(self):
        self._k, sub = jax.random.split(self._k)
        return sub

    def normal(self, shape):
        return jax.random.normal(self._next(), shape, dtype=jnp.bfloat16)

    def randint(self, lo, hi, shape):
        return jax.random.randint(self._next(), shape, lo, hi, dtype=jnp.int32)

    def uniform(self, shape, lo=0.0, hi=1.0):
        return jax.random.uniform(self._next(), shape, jnp.bfloat16, lo, hi)

    def permutation(self, n):
        return jax.random.permutation(self._next(), n)
kernel_name = 'adaLN_cond__sliding_block_cached__mixer_channel_mlp__decode'

def setup_inputs():
    _rng = _Rng(jax.random.key(int.from_bytes(__import__("os").urandom(4), "little")))
    _w = lambda a: (lambda t: t.astype(jnp.bfloat16) if jnp.issubdtype(t.dtype, jnp.floating) else t)(jnp.asarray(a))

    def _A_setup():
        B, Sq, D = (8, 1, 640)
        Hq, Hkv, Sk, Dh = (32, 32, 4096, 192)
        assert Hq % Hkv == 0, (Hq, Hkv)
        return {'x': _w((lambda *s: _rng.normal(s) * 0.05)(B, Sq, D)), 'k_cache': _w((lambda *s: _rng.normal(s) * 0.05)(B, Hkv, Sk, Dh)), 'v_cache': _w((lambda *s: _rng.normal(s) * 0.05)(B, Hkv, Sk, Dh)), 'wq': _w((lambda *s: _rng.normal(s) * 0.05)(D, Hq * Dh) * D ** (-0.5)), 'wo': _w((lambda *s: _rng.normal(s) * 0.05)(Hq * Dh, D) * (Hq * Dh) ** (-0.5))}
    _A_in = _A_setup()

    def _B_setup():
        B, S, D, F = (8, 1, 640, 1536)
        return {'x': _w((lambda *s: _rng.normal(s) * 0.05)(B, S, D)), 'w1': _w((lambda *s: _rng.normal(s) * 0.05)(D, F) * D ** (-0.5)), 'b1': _w((lambda *s: _rng.normal(s) * 0.05)(F)), 'w2': _w((lambda *s: _rng.normal(s) * 0.05)(F, D) * F ** (-0.5)), 'b2': _w((lambda *s: _rng.normal(s) * 0.05)(D))}
    _B_in = _B_setup()
    return {'A_x': _A_in['x'], 'A_k_cache': _A_in['k_cache'], 'A_v_cache': _A_in['v_cache'], 'A_wq': _A_in['wq'], 'A_wo': _A_in['wo'], 'B_x': _B_in['x'], 'B_w1': _B_in['w1'], 'B_b1': _B_in['b1'], 'B_w2': _B_in['w2'], 'B_b2': _B_in['b2'], 'c': _w((lambda *s: _rng.normal(s) * 0.05)(8, 640)), 'w_mod': _w((lambda *s: _rng.normal(s) * 0.05)(640, 6 * 640) * 640 ** (-0.5))}

def reference(A_x, A_k_cache, A_v_cache, A_wq, A_wo, B_x, B_w1, B_b1, B_w2, B_b2, c, w_mod):

    def _A_ref(x, k_cache, v_cache, wq, wo):
        B, Sq, D = x.shape
        Hq, Dh = (32, 192)
        Hkv, Sk = (k_cache.shape[1], k_cache.shape[2])
        W = min(4096, max(256, Sk // 4))
        rep = Hq // Hkv
        q = (lambda x, *d: x.transpose(*d))((x @ wq).reshape(B, Sq, Hq, Dh), 0, 2, 1, 3)
        k = jnp.repeat(k_cache[:, :, Sk - W:, :], rep, axis=1)
        v = jnp.repeat(v_cache[:, :, Sk - W:, :], rep, axis=1)
        scores = jnp.einsum('bhqd,bhkd->bhqk', q, k) * Dh ** (-0.5)
        p = _softmax(scores, axis=-1)
        o = jnp.einsum('bhqk,bhkd->bhqd', p, v)
        return (lambda x, *d: x.transpose(*d))(o, 0, 2, 1, 3).reshape(B, Sq, Hq * Dh) @ wo

    def _B_ref(x, w1, b1, w2, b2):
        y = _layernorm(x, axis=-1)
        h = _gelu(jnp.einsum('bsd,df->bsf', y, w1) + b1)
        return jnp.einsum('bsf,fd->bsd', h, w2) + b2
    x = A_x
    mod = (_silu(c) @ w_mod).reshape(c.shape[0], 6, 1, -1)
    sa, ca, ga, sb, cb, gb = (mod[:, 0].copy(), mod[:, 1].copy(), mod[:, 2].copy(), mod[:, 3].copy(), mod[:, 4].copy(), mod[:, 5].copy())
    h = _layernorm(x, axis=-1) * (1 + ca) + sa
    x = x + ga * _A_ref(h, A_k_cache, A_v_cache, A_wq, A_wo)
    h = _layernorm(x, axis=-1) * (1 + cb) + sb
    x = x + gb * _B_ref(h, B_w1, B_b1, B_w2, B_b2)
    return x
```

```python
import jax
import jax.numpy as jnp
from jax import lax
import jax.experimental.pallas as pl
import jax.experimental.pallas.tpu as pltpu

EPS = 1e-5
NUM_HEADS = 32
NBUF = 3
ROWS = 8

f32, bf16 = jnp.float32, jnp.bfloat16


def _layernorm(x):
    m = jnp.mean(x, axis=-1, keepdims=True)
    xc = x - m
    v = jnp.mean(xc * xc, axis=-1, keepdims=True)
    return xc / jnp.sqrt(v + EPS)


def _interleave(compute, dmas):
    n = len(compute)
    for i, fn in enumerate(compute):
        for d in dmas[len(dmas) * i // n: len(dmas) * (i + 1) // n]:
            d()
        fn()


def _kernel(x_hbm, c_hbm, b1_hbm, b2_hbm, k_hbm, v_hbm, wq_hbm, wo_hbm, w1_hbm, w2_hbm, wm_hbm,
            o_ref,
            kb, vb, wq_v, wo_v, w1_v, w2_v, wm_v, x_v, c_v, b1_v, b2_v, q_s, o_s, mod_s,
            kv_sem, w_sem):
    B, H, DH, S = k_hbm.shape
    W = kb.shape[-1]
    D = x_v.shape[-1]
    F = b1_v.shape[0]

    def kv_dmas(h, slot):
        out = []
        for r in range(0, DH, ROWS):
            for b in range(B):
                for a, (src, dst) in enumerate(((k_hbm, kb), (v_hbm, vb))):
                    def go(r=r, b=b, a=a, src=src, dst=dst):
                        pltpu.make_async_copy(
                            src.at[b, h, pl.ds(r, ROWS), pl.ds(S - W, W)],
                            dst.at[slot, b, pl.ds(r, ROWS), :],
                            kv_sem.at[a, slot]).start(priority=a)
                    out.append(go)
        return out

    def w_dmas(src, dst, sem, rows, cols):
        out = []
        for r in range(0, src.shape[0], rows):
            for c0 in range(0, src.shape[1], cols):
                def go(r=r, c0=c0, j=len(out)):
                    pltpu.make_async_copy(src.at[pl.ds(r, rows), pl.ds(c0, cols)],
                                          dst.at[pl.ds(r, rows), pl.ds(c0, cols)],
                                          w_sem.at[sem]).start(priority=j % 2)
                out.append(go)
        return out

    def wait_all(dst, sem):
        pltpu.make_async_copy(dst, dst, sem).wait()

    small = [pltpu.make_async_copy(s, d, w_sem.at[i]) for i, (s, d) in enumerate(
        ((c_hbm, c_v), (x_hbm, x_v), (b1_hbm, b1_v), (b2_hbm, b2_v)))]
    SEM_WM, SEM_WQ, SEM_WO, SEM_W1, SEM_W2 = 4, 5, 6, 7, 8
    for cp in small:
        cp.start()
    for d in w_dmas(wm_hbm, wm_v, SEM_WM, 8, 768):
        d()
    for d in w_dmas(wq_hbm, wq_v, SEM_WQ, 8, 1024):
        d()
    for cp in small:
        cp.wait()
    wait_all(wm_v, w_sem.at[SEM_WM])

    cf = c_v[...].astype(f32)
    sc = (cf * jax.nn.sigmoid(cf)).astype(bf16)

    def mod_chunk(j):
        def go():
            mod_s[j] = jnp.dot(sc, wm_v[:, j * D:(j + 1) * D], preferred_element_type=f32)
        return go
    _interleave([mod_chunk(j) for j in range(6)], kv_dmas(0, 0))

    xf = x_v[...].astype(f32)
    h1 = (_layernorm(xf) * (1.0 + mod_s[1]) + mod_s[0]).astype(bf16)
    wait_all(wq_v, w_sem.at[SEM_WQ])

    def q_chunk(p):
        def go():
            qq = jnp.dot(h1, wq_v[:, p * 2 * DH:(p + 1) * 2 * DH], preferred_element_type=f32)
            q_s[2 * p] = qq[:, :DH]
            q_s[2 * p + 1] = qq[:, DH:]
        return go
    pro = []
    for s in range(1, NBUF - 1):
        pro += kv_dmas(s, s)
    _interleave([q_chunk(p) for p in range(H // 2)], pro)

    row = lax.broadcasted_iota(jnp.int32, (B, 1), 0)

    def attend(h, slot, dmas):
        st = {}
        q = q_s[h].astype(bf16)

        def qk(b):
            def go():
                if b == 0:
                    wait_all(kb.at[slot], kv_sem.at[0, slot])
                s = jnp.dot(q, kb[slot, b], preferred_element_type=f32)
                st['s'] = s if b == 0 else jnp.where(row == b, s, st['s'])
            return go

        def pv(b):
            def go():
                if b == 0:
                    wait_all(vb.at[slot], kv_sem.at[1, slot])
                    s = st['s'] * (DH ** -0.5)
                    e = jnp.exp(s - jnp.max(s, axis=-1, keepdims=True))
                    st['l'] = jnp.sum(e, axis=-1, keepdims=True)
                    st['p'] = e.astype(bf16)
                o = lax.dot_general(st['p'], vb[slot, b], (((1,), (1,)), ((), ())),
                                    preferred_element_type=f32)
                st['o'] = o if b == 0 else jnp.where(row == b, o, st['o'])
                if b == B - 1:
                    o_s[h] = st['o'] / st['l']
            return go
        _interleave([qk(b) for b in range(B)] + [pv(b) for b in range(B)], dmas)

    def body(h, carry):
        nxt = h + (NBUF - 1)
        attend(h, h % NBUF, kv_dmas(nxt, nxt % NBUF))
        return carry
    n_main = H - (NBUF - 1)
    lax.fori_loop(0, n_main, body, 0)

    tail = (w_dmas(wo_hbm, wo_v, SEM_WO, 16, D) + w_dmas(w1_hbm, w1_v, SEM_W1, 8, 768)
            + w_dmas(w2_hbm, w2_v, SEM_W2, 16, D))
    nt = NBUF - 1
    for i in range(nt):
        h = n_main + i
        attend(h, h % NBUF, tail[len(tail) * i // nt: len(tail) * (i + 1) // nt])

    wait_all(wo_v, w_sem.at[SEM_WO])
    attn = jnp.zeros((B, D), f32)
    for p in range(H // 2):
        oo = jnp.concatenate([o_s[2 * p], o_s[2 * p + 1]], axis=-1).astype(bf16)
        attn += jnp.dot(oo, wo_v[p * 2 * DH:(p + 1) * 2 * DH, :], preferred_element_type=f32)
    x1 = xf + mod_s[2] * attn
    h2 = _layernorm(x1) * (1.0 + mod_s[4]) + mod_s[3]
    y = _layernorm(h2).astype(bf16)
    wait_all(w1_v, w_sem.at[SEM_W1])
    u = jnp.dot(y, w1_v[...], preferred_element_type=f32) + b1_v[...].astype(f32).reshape(1, F)
    g = jax.nn.gelu(u, approximate=True).astype(bf16)
    wait_all(w2_v, w_sem.at[SEM_W2])
    mlp = jnp.dot(g, w2_v[...], preferred_element_type=f32) + b2_v[...].astype(f32).reshape(1, D)
    o_ref[...] = (x1 + mod_s[5] * mlp).astype(o_ref.dtype)


@jax.jit
def pallas_adaLN_cond__sliding_block_cached__mixer_channel_mlp__decode_kernel(
    A_x: jax.Array,
    A_k_cache: jax.Array,
    A_v_cache: jax.Array,
    A_wq: jax.Array,
    A_wo: jax.Array,
    B_x: jax.Array,
    B_w1: jax.Array,
    B_b1: jax.Array,
    B_w2: jax.Array,
    B_b2: jax.Array,
    c: jax.Array,
    w_mod: jax.Array,
):
    del B_x
    B, Sq, D = A_x.shape
    _, H, S, DH = A_k_cache.shape
    F = B_w1.shape[1]
    assert Sq == 1 and H == NUM_HEADS
    W = min(4096, max(256, S // 4))
    kt = jnp.transpose(A_k_cache, (0, 1, 3, 2))
    vt = jnp.transpose(A_v_cache, (0, 1, 3, 2))
    out = pl.pallas_call(
        _kernel,
        in_specs=[pl.BlockSpec(memory_space=pltpu.HBM)] * 11,
        out_specs=pl.BlockSpec(memory_space=pltpu.VMEM),
        out_shape=jax.ShapeDtypeStruct((B, D), A_x.dtype),
        scratch_shapes=[
            pltpu.VMEM((NBUF, B, DH, W), bf16), pltpu.VMEM((NBUF, B, DH, W), bf16),
            pltpu.VMEM(A_wq.shape, bf16), pltpu.VMEM(A_wo.shape, bf16),
            pltpu.VMEM(B_w1.shape, bf16), pltpu.VMEM(B_w2.shape, bf16),
            pltpu.VMEM(w_mod.shape, bf16),
            pltpu.VMEM((B, D), bf16), pltpu.VMEM((B, D), bf16),
            pltpu.VMEM((F,), bf16), pltpu.VMEM((D,), bf16),
            pltpu.VMEM((H, B, DH), f32), pltpu.VMEM((H, B, DH), f32), pltpu.VMEM((6, B, D), f32),
            pltpu.SemaphoreType.DMA((2, NBUF)), pltpu.SemaphoreType.DMA((9,)),
        ],
        compiler_params=pltpu.CompilerParams(vmem_limit_bytes=100 * 2**20),
    )(A_x.reshape(B, D), c, B_b1, B_b2, kt, vt, A_wq, A_wo, B_w1, B_w2, w_mod)
    return out.reshape(B, Sq, D)
```

```python
import jax
import jax.numpy as jnp
from jax import lax
import jax.experimental.pallas as pl
import jax.experimental.pallas.tpu as pltpu

EPS = 1e-5
NUM_SLOTS = 3
TILE_ROWS = 8
NUM_STREAMS = 8
WO_LAG = 192
W2_SPLIT = (6, 3, 2, 1)

f32, bf16 = jnp.float32, jnp.bfloat16


def _layernorm(x):
    m = jnp.mean(x, axis=-1, keepdims=True)
    xc = x - m
    v = jnp.mean(xc * xc, axis=-1, keepdims=True)
    return xc / jnp.sqrt(v + EPS)


class _Stream:
    def __init__(self, copies):
        self.copies = copies
        self.pos = 0

    def start_until(self, n):
        while self.pos < min(n, len(self.copies)):
            make_copy, priority = self.copies[self.pos]
            make_copy().start(priority=priority)
            self.pos += 1

    def interleave(self, tasks, until=None):
        until = len(self.copies) if until is None else until
        first = self.pos
        for i, task in enumerate(tasks):
            self.start_until(first + (until - first) * (i + 1) // len(tasks))
            task()


def _wait_filled(buf, sem):
    pltpu.make_async_copy(buf, buf, sem).wait()


def _weight_copies(src, dst, sem, rows, cols, row_range=None):
    r0, r1 = row_range or (0, src.shape[0])
    ncols = src.shape[1]
    pieces = [(r, c, min(cols, ncols - c))
              for r in range(r0, r1, rows) for c in range(0, ncols, cols)]
    per = -(-len(pieces) // NUM_STREAMS)
    order = [t * per + i for i in range(per) for t in range(NUM_STREAMS)
             if t * per + i < len(pieces)]

    def piece(r, c, n):
        idx = (pl.ds(r, rows), pl.ds(c, n))
        return lambda: pltpu.make_async_copy(src.at[idx], dst.at[idx], sem)

    return [(piece(*pieces[k]), (j // 2) % 2) for j, k in enumerate(order)]


def _kernel(x_hbm, c_hbm, b1_hbm, b2_hbm, k_hbm, v_hbm, wq_hbm, wo_hbm, w1_hbm, w2_hbm, wm_hbm,
            out_ref,
            kv_buf, wq_buf, wo_buf, w1_buf, w2_buf, wm_buf, x_buf, c_buf, b1_buf, b2_buf,
            q_scr, o_scr, mod_scr, sems):
    B, H, DH, S = k_hbm.shape
    W = kv_buf.shape[-1]
    D = x_buf.shape[-1]
    F = b1_buf.shape[0]

    def kv_sem(a, h):
        return sems.at[2 + h % NUM_SLOTS if a else h % 2]

    def kv_copies(h):
        slot = h % NUM_SLOTS

        def strip(a, src, b, r):
            return lambda: pltpu.make_async_copy(
                src.at[pl.ds(b, 2), h, pl.ds(r, TILE_ROWS), pl.ds(S - W, W)],
                kv_buf.at[a, slot, pl.ds(b, 2), pl.ds(r, TILE_ROWS), :],
                kv_sem(a, h))

        return [(strip(a, src, b, r), a)
                for r in range(0, DH, TILE_ROWS)
                for b in range(0, B, 2)
                for a, src in enumerate((k_hbm, v_hbm))]

    small = [pltpu.make_async_copy(src, dst, kv_sem(0, 0)) for src, dst in (
        (c_hbm, c_buf), (x_hbm, x_buf), (b1_hbm, b1_buf), (b2_hbm, b2_buf))]
    for copy in small:
        copy.start()
    wm_sem, wq_sem = kv_sem(1, 0), kv_sem(0, 1)
    head = _Stream(_weight_copies(wm_hbm, wm_buf, wm_sem, TILE_ROWS, 1024)
                   + _weight_copies(wq_hbm, wq_buf, wq_sem, TILE_ROWS, 1024))
    head.start_until(len(head.copies))
    for copy in small:
        copy.wait()
    _wait_filled(wm_buf, wm_sem)

    c = c_buf[...].astype(f32)
    c_act = (c * jax.nn.sigmoid(c)).astype(bf16)

    def mod_task(j):
        def run():
            mod_scr[j] = jnp.dot(c_act, wm_buf[:, j * D:(j + 1) * D], preferred_element_type=f32)
        return run

    _Stream(kv_copies(0)).interleave([mod_task(j) for j in range(6)])

    x = x_buf[...].astype(f32)
    h_attn = (_layernorm(x) * (1.0 + mod_scr[1]) + mod_scr[0]).astype(bf16)
    _wait_filled(wq_buf, wq_sem)

    def q_task(p):
        def run():
            q = jnp.dot(h_attn, wq_buf[:, 2 * p * DH:2 * (p + 1) * DH], preferred_element_type=f32)
            q_scr[2 * p] = q[:, :DH]
            q_scr[2 * p + 1] = q[:, DH:]
        return run

    _Stream(kv_copies(1)).interleave([q_task(p) for p in range(H // 2)])

    row = lax.broadcasted_iota(jnp.int32, (B, 1), 0)

    def attention_tasks(h):
        slot = h % NUM_SLOTS
        _wait_filled(kv_buf.at[0, slot], kv_sem(0, h))
        q = q_scr[h].astype(bf16)
        state = {}

        def keep(name, b, value):
            state[name] = value if b == 0 else jnp.where(row == b, value, state[name])

        def qk_task(b):
            def run():
                keep('s', b, jnp.dot(q, kv_buf[0, slot, b], preferred_element_type=f32))
            return run

        def pv_task(b):
            def run():
                if b == 0:
                    _wait_filled(kv_buf.at[1, slot], kv_sem(1, h))
                    s = state['s'] * (DH ** -0.5)
                    e = jnp.exp(s - jnp.max(s, axis=-1, keepdims=True))
                    state['l'] = jnp.sum(e, axis=-1, keepdims=True)
                    state['p'] = e.astype(bf16)
                keep('o', b, lax.dot_general(state['p'], kv_buf[1, slot, b],
                                             (((1,), (1,)), ((), ())),
                                             preferred_element_type=f32))
                if b == B - 1:
                    o_scr[h] = state['o'] / state['l']
            return run

        return [qk_task(b) for b in range(B)] + [pv_task(b) for b in range(B)]

    def head_step(h, carry):
        tasks = attention_tasks(h)
        _Stream(kv_copies(h + 2)).interleave(tasks)
        return carry

    lax.fori_loop(0, H - 2, head_step, 0)

    wo_sem = kv_sem(1, H - 3)
    w1_sem = kv_sem(0, H - 2)
    w2_sems = (kv_sem(0, H - 1), kv_sem(1, H - 2), kv_sem(1, H - 1), wo_sem)
    bounds = [F * sum(W2_SPLIT[:i]) // sum(W2_SPLIT) for i in range(len(W2_SPLIT) + 1)]
    copies = _weight_copies(wo_hbm, wo_buf, wo_sem, 2 * TILE_ROWS, D)
    n_wo = len(copies)
    copies += _weight_copies(w1_hbm, w1_buf, w1_sem, TILE_ROWS, F // 2)
    for lo, hi, sem in zip(bounds, bounds[1:], w2_sems):
        last_piece = len(copies)
        copies += _weight_copies(w2_hbm, w2_buf, sem, 2 * TILE_ROWS, D, (lo, hi))
    tail = _Stream(copies)
    tail.interleave(attention_tasks(H - 2), until=n_wo // 2)
    tail.interleave(attention_tasks(H - 1), until=n_wo)

    tail.start_until(min(n_wo + WO_LAG, last_piece))
    _wait_filled(wo_buf, wo_sem)
    attn = jnp.zeros((B, D), f32)
    for p in range(H // 2):
        o = jnp.concatenate([o_scr[2 * p], o_scr[2 * p + 1]], axis=-1).astype(bf16)
        attn += jnp.dot(o, wo_buf[2 * p * DH:2 * (p + 1) * DH, :], preferred_element_type=f32)
        tail.start_until(tail.pos + 2)
    x = x + mod_scr[2] * attn

    h_mlp = _layernorm(x) * (1.0 + mod_scr[4]) + mod_scr[3]
    y = _layernorm(h_mlp).astype(bf16)
    tail.start_until(len(copies))
    _wait_filled(w1_buf, w1_sem)
    u = jnp.dot(y, w1_buf[...], preferred_element_type=f32) + b1_buf[...].astype(f32).reshape(1, F)
    g = jax.nn.gelu(u, approximate=True).astype(bf16)
    mlp = b2_buf[...].astype(f32).reshape(1, D)
    for lo, hi, sem in zip(bounds, bounds[1:], w2_sems):
        part = w2_buf.at[pl.ds(lo, hi - lo)]
        _wait_filled(part, sem)
        mlp = mlp + jnp.dot(g[:, lo:hi], part[...], preferred_element_type=f32)
    out_ref[...] = (x + mod_scr[5] * mlp).astype(out_ref.dtype)


@jax.jit
def pallas_adaLN_cond__sliding_block_cached__mixer_channel_mlp__decode_kernel(
    A_x: jax.Array,
    A_k_cache: jax.Array,
    A_v_cache: jax.Array,
    A_wq: jax.Array,
    A_wo: jax.Array,
    B_x: jax.Array,
    B_w1: jax.Array,
    B_b1: jax.Array,
    B_w2: jax.Array,
    B_b2: jax.Array,
    c: jax.Array,
    w_mod: jax.Array,
):
    del B_x
    B, Sq, D = A_x.shape
    _, H, S, DH = A_k_cache.shape
    F = B_w1.shape[1]
    assert Sq == 1 and A_wq.shape == (D, H * DH)
    W = min(4096, max(256, S // 4))
    k_t = jnp.transpose(A_k_cache, (0, 1, 3, 2))
    v_t = jnp.transpose(A_v_cache, (0, 1, 3, 2))
    out = pl.pallas_call(
        _kernel,
        in_specs=[pl.BlockSpec(memory_space=pltpu.HBM)] * 11,
        out_specs=pl.BlockSpec(memory_space=pltpu.VMEM),
        out_shape=jax.ShapeDtypeStruct((B, D), A_x.dtype),
        scratch_shapes=[
            pltpu.VMEM((2, NUM_SLOTS, B, DH, W), A_k_cache.dtype),
            pltpu.VMEM(A_wq.shape, A_wq.dtype),
            pltpu.VMEM(A_wo.shape, A_wo.dtype),
            pltpu.VMEM(B_w1.shape, B_w1.dtype),
            pltpu.VMEM(B_w2.shape, B_w2.dtype),
            pltpu.VMEM(w_mod.shape, w_mod.dtype),
            pltpu.VMEM((B, D), A_x.dtype),
            pltpu.VMEM(c.shape, c.dtype),
            pltpu.VMEM(B_b1.shape, B_b1.dtype),
            pltpu.VMEM(B_b2.shape, B_b2.dtype),
            pltpu.VMEM((H, B, DH), f32),
            pltpu.VMEM((H, B, DH), f32),
            pltpu.VMEM((6, B, D), f32),
            pltpu.SemaphoreType.DMA((2 + NUM_SLOTS,)),
        ],
        compiler_params=pltpu.CompilerParams(vmem_limit_bytes=64 * 2**20),
    )(A_x.reshape(B, D), c, B_b1, B_b2, k_t, v_t, A_wq, A_wo, B_w1, B_w2, w_mod)
    return out.reshape(B, Sq, D)
```
